```python
import os as _os
_os.environ.setdefault("JAX_PLATFORMS", "cpu")
import jax
import jax.numpy as jnp

def _softmax(x, axis=-1):
    return jax.nn.softmax(x, axis=axis)
def _gelu(x):
    return jax.nn.gelu(x, approximate=True)
def _silu(x):
    return jax.nn.silu(x)
def _sigmoid(x):
    return jax.nn.sigmoid(x)
def _layernorm(x, axis=-1, eps=1e-5):
    m = jnp.mean(x, axis=axis, keepdims=True)
    v = jnp.var(x, axis=axis, keepdims=True)
    return (x - m) / jnp.sqrt(v + eps)
def _scatter_add(tgt, idx, src, axis=0):
    return tgt.at[idx].add(src)
def _segment_sum(src, seg, n):
    return jax.ops.segment_sum(src, seg, n)
class _Rng:
    def __init__(self, key):
        self._k = key
    def _next(self):
        self._k, sub = jax.random.split(self._k)
        return sub
    def normal(self, shape):
        return jax.random.normal(self._next(), shape, dtype=jnp.bfloat16)
    def randint(self, lo, hi, shape):
        return jax.random.randint(self._next(), shape, lo, hi, dtype=jnp.int32)
    def uniform(self, shape, lo=0.0, hi=1.0):
        return jax.random.uniform(self._next(), shape, jnp.bfloat16, lo, hi)
    def permutation(self, n):
        return jax.random.permutation(self._next(), n)


kernel_name = 'interleave_layers__grouped_kv_mqa__sliding_block__prompt'

def setup_inputs():
    _rng = _Rng(jax.random.key(int.from_bytes(__import__("os").urandom(4), "little")))
    _w = (lambda a: (lambda t: t.astype(jnp.bfloat16) if jnp.issubdtype(t.dtype, jnp.floating) else t)(jnp.asarray(a)))
    def _A_setup():
        B, S, D, H = 1, 2048, 448, 16
        Dh = D // H
        return {
            "x": _w((lambda *s: _rng.normal(s) * 0.05)(B, S, D)),
            "wq": _w((lambda *s: _rng.normal(s) * 0.05)(D, H * Dh)),
            "wk": _w((lambda *s: _rng.normal(s) * 0.05)(D, Dh)),
            "wv": _w((lambda *s: _rng.normal(s) * 0.05)(D, Dh)),
            "wo": _w((lambda *s: _rng.normal(s) * 0.05)(H * Dh, D)),
        }
    _A_in = _A_setup()

    def _B_setup():
        B, S, D = 1, 2048, 448
        return {
            "x": _w((lambda *s: _rng.normal(s) * 0.05)(B, S, D)),
            "wqkv": _w((lambda *s: _rng.normal(s) * 0.05)(D, 3 * D)),
            "wo": _w((lambda *s: _rng.normal(s) * 0.05)(D, D)),
        }
    _B_in = _B_setup()

    return {
        "A_x": _A_in["x"],
        "A_wq": _A_in["wq"],
        "A_wk": _A_in["wk"],
        "A_wv": _A_in["wv"],
        "A_wo": _A_in["wo"],
        "B_x": _B_in["x"],
        "B_wqkv": _B_in["wqkv"],
        "B_wo": _B_in["wo"],
    }

def reference(A_x, A_wq, A_wk, A_wv, A_wo, B_x, B_wqkv, B_wo):
    def _A_ref(x, wq, wk, wv, wo):
        B, S, D = x.shape
        H = 16
        Dh = D // H
        q = (lambda x, *d: x.transpose(*d))((x @ wq).reshape(B, S, H, Dh), 0, 2, 1, 3)
        k = x @ wk
        v = x @ wv
        scores = jnp.einsum("bhqd,bkd->bhqk", q, k) * (Dh ** -0.5)
        p = _softmax(scores, axis=-1)
        o = jnp.einsum("bhqk,bkd->bhqd", p, v)
        return (lambda x, *d: x.transpose(*d))(o, 0, 2, 1, 3).reshape(B, S, H * Dh) @ wo

    def _B_ref(x, wqkv, wo):
        B, S, D = x.shape
        H = 16; Dh = D // H; W = 256
        qkv = (lambda x, *d: x.transpose(*d))((x @ wqkv).reshape(B, S, 3, H, Dh), 2, 0, 3, 1, 4)
        q, k, v = qkv[0], qkv[1], qkv[2]
        scores = jnp.einsum("bhqd,bhkd->bhqk", q, k) * (Dh ** -0.5)
        idx = jnp.arange(S)
        mask = (idx[:, None] - idx[None, :] >= 0) & (idx[:, None] - idx[None, :] < W)
        scores = jnp.where(mask[None, None], scores, -1e9)
        p = _softmax(scores, axis=-1)
        o = jnp.einsum("bhqk,bhkd->bhqd", p, v)
        return (lambda x, *d: x.transpose(*d))(o, 0, 2, 1, 3).reshape(B, S, D) @ wo

    x = A_x
    x = x + _A_ref(_layernorm(x, axis=-1), A_wq, A_wk, A_wv, A_wo)
    x = x + _B_ref(_layernorm(x, axis=-1), B_wqkv, B_wo)
    x = x + _A_ref(_layernorm(x, axis=-1), A_wq, A_wk, A_wv, A_wo)
    x = x + _B_ref(_layernorm(x, axis=-1), B_wqkv, B_wo)
    return x
```

```python
import functools
import math

import jax
import jax.numpy as jnp
from jax import lax
import jax.experimental.pallas as pl
import jax.experimental.pallas.tpu as pltpu

S = 2048
D = 448
H = 16
DH = 28
HP = 32
DP = H * HP
W = 256
EPS = 1e-5
QSCALE = (DH ** -0.5) * math.log2(math.e)
NEG = -1e30

TB = 512
NQ = 512
KC = 128
UA = 4
UB = 2
KW = W + 128
F32 = jnp.float32
BF16 = jnp.bfloat16
U32 = jnp.uint32


def _nn(a, b):
    return jnp.dot(a, b, preferred_element_type=F32)


def _nt(a, b):
    return lax.dot_general(a, b, (((1,), (1,)), ((), ())), preferred_element_type=F32)


def _tn(a, b):
    return lax.dot_general(a, b, (((0,), (0,)), ((), ())), preferred_element_type=F32)


def _sel_T(b, a, width):
    p = lax.broadcasted_iota(jnp.int32, (128, width), 0)
    c = lax.broadcasted_iota(jnp.int32, (128, width), 1)
    d = p & 31
    src = 112 * b + 28 * (p >> 5) + d - a
    return jnp.where((c == src) & (d < DH), 1.0, 0.0).astype(BF16)


def _pad_transpose_into(dst_ref, row0, w_ref, nblocks, ncols):
    for b in range(nblocks):
        a = (112 * b // 128) * 128
        width = min(256, ncols - a)
        res = _nt(_sel_T(b, a, width), w_ref[:, a:a + width])
        dst_ref[row0 + 128 * b: row0 + 128 * (b + 1), :] = res.astype(BF16)


def _wo_transpose_into(dst_ref, wo_ref):
    r = lax.broadcasted_iota(jnp.int32, (112, 128), 0)
    p = lax.broadcasted_iota(jnp.int32, (112, 128), 1)
    d = p & 31
    e = jnp.where((r == 28 * (p >> 5) + d) & (d < DH), 1.0, 0.0).astype(BF16)
    for g in range(4):
        res = _tn(wo_ref[112 * g:112 * (g + 1), :], e)
        dst_ref[:, 128 * g:128 * (g + 1)] = res.astype(BF16)


def _layernorm_T(xt):
    m = jnp.sum(xt, axis=0, keepdims=True) * (1.0 / D)
    xc = xt - m
    v = jnp.sum(xc * xc, axis=0, keepdims=True) * (1.0 / D)
    return (xc * lax.rsqrt(v + EPS)).astype(BF16)


def _kernel(x_ref, awq_ref, awk_ref, awv_ref, awo_ref, bwqkv_ref, bwo_ref, o_ref,
            xT, wA, woA, wB, woB, qT, kA, vA, kB, vB, oT, s_ref, m_ref, p_ref, mB_ref):
    _pad_transpose_into(wA, 0, awq_ref, 4, D)
    eye = jnp.where(lax.broadcasted_iota(jnp.int32, (HP, DH), 0)
                    == lax.broadcasted_iota(jnp.int32, (HP, DH), 1), 1.0, 0.0).astype(BF16)
    wA[DP:DP + HP, :] = _nn(eye, awk_ref[...]).astype(BF16)
    wA[DP + HP:DP + 2 * HP, :] = _nn(eye, awv_ref[...]).astype(BF16)
    _wo_transpose_into(woA, awo_ref)
    _pad_transpose_into(wB, 0, bwqkv_ref, 12, 3 * D)
    _wo_transpose_into(woB, bwo_ref)

    nb = S // TB

    def tok(i):
        return pl.ds(pl.multiple_of(i * TB, TB), TB)

    def tokh(i):
        return pl.ds(pl.multiple_of(i * (TB // 2), TB // 2), TB // 2)

    def load_x(i, c):
        xT[:, tok(i)] = x_ref[:, tok(i)].astype(F32)
        return c
    lax.fori_loop(0, nb, load_x, 0)

    ones_row_A = lax.broadcasted_iota(jnp.int32, (HP, TB), 0) == DH
    ones_row_B = (lax.broadcasted_iota(jnp.int32, (DP, TB), 0) & 31) == DH

    def proj_A(i):
        xn = _layernorm_T(xT[:, tok(i)])
        r = _nn(wA[...], xn)
        qT[:, tok(i)] = (r[0:DP] * QSCALE).astype(BF16)
        kA[tokh(i), :] = pltpu.bitcast(r[DP:DP + HP].T.astype(BF16), U32)
        vA[:, tok(i)] = jnp.where(ones_row_A, 1.0, r[DP + HP:DP + 2 * HP]).astype(BF16)

    def proj_B(i):
        xn = _layernorm_T(xT[:, tok(i)])
        r = _nn(wB[...], xn)
        qT[:, tok(i)] = (r[0:DP] * QSCALE).astype(BF16)
        kB[tokh(i), :] = pltpu.bitcast(r[DP:2 * DP].astype(BF16).T, U32)
        vB[:, tok(i)] = jnp.where(ones_row_B, 1.0, r[2 * DP:3 * DP]).astype(BF16)

    def out_proj(i, wo):
        xT[:, tok(i)] = xT[:, tok(i)] + _nn(wo[...], oT[:, tok(i)])

    nqb = S // NQ
    nblk = H * nqb
    nch = S // KC

    def blk_slices(b):
        j = b // H
        h = b % H
        if isinstance(b, int):
            return pl.ds(h * HP, HP), pl.ds(j * NQ, NQ)
        return (pl.ds(pl.multiple_of(h * HP, HP), HP), pl.ds(pl.multiple_of(j * NQ, 128), NQ))

    def a_stage(bpv, do_ex, bqk, par):
        m_old = m_ref[...] if do_ex else None
        q = qT[blk_slices(bqk)] if bqk is not None else None
        o = None
        m8 = None
        for c in range(nch):
            rows = slice(c * KC, (c + 1) * KC)
            prow = slice(c * KC // 2, (c + 1) * KC // 2)
            if bpv is not None:
                oc = _nn(vA[:, rows], pltpu.bitcast(p_ref.at[1 - par][prow], BF16))
                o = oc if o is None else o + oc
            if do_ex:
                p = jnp.exp2(s_ref[rows] - m_old).astype(BF16)
                p_ref.at[par][prow] = pltpu.bitcast(p, U32)
            if bqk is not None:
                s = _nn(pltpu.bitcast(kA[prow], BF16), q)
                s_ref[rows] = s
                mc = jnp.max(s.reshape(KC // 8, 8, NQ), axis=0)
                m8 = mc if m8 is None else jnp.maximum(m8, mc)
        if bqk is not None:
            m_ref[...] = jnp.max(m8, axis=0, keepdims=True)
        if bpv is not None:
            oT[blk_slices(bpv)] = (o / o[DH:DH + 1, :]).astype(BF16)

    def attn_A():
        npeel = (nblk - 2) % UA
        a_stage(None, False, 0, 1)
        a_stage(None, True, 1, 0)
        for b in range(1, 1 + npeel):
            a_stage(b - 1, True, b + 1, b % 2)

        def body(i, c):
            for u in range(UA):
                b = 1 + npeel + i * UA + u
                a_stage(b - 1, True, b + 1, (1 + npeel + u) % 2)
            return c
        lax.fori_loop(0, (nblk - 2 - npeel) // UA, body, 0)
        a_stage(nblk - 2, True, None, (nblk - 1) % 2)
        a_stage(nblk - 1, False, None, nblk % 2)

    def attn_B():
        r = lax.broadcasted_iota(jnp.int32, (128, DP), 0)
        c = lax.broadcasted_iota(jnp.int32, (128, DP), 1) & 127
        lower = r > c

        def ntile(t):
            return min(t + 1, 3) if isinstance(t, int) else 3

        def off(t, n, div=1):
            if isinstance(t, int):
                return (t + 1 - n) * 128 // div
            return pl.multiple_of((t + 1 - n) * (128 // div), 128 // div)

        def qsl(t):
            return pl.ds(t * 128, 128) if isinstance(t, int) else pl.ds(pl.multiple_of(t * 128, 128), 128)

        def wq_of(t, g):
            qg = qT[128 * g:128 * (g + 1), qsl(t)]
            cols = []
            for i in range(4):
                parts = []
                if i > 0:
                    parts.append(jnp.zeros((HP * i, 128), BF16))
                parts.append(qg[HP * i:HP * (i + 1)])
                if i < 3:
                    parts.append(jnp.zeros((HP * (3 - i), 128), BF16))
                cols.append(jnp.concatenate(parts, axis=0))
            return jnp.concatenate(cols, axis=1)

        def qk(t, g):
            n = ntile(t)
            kk = pltpu.bitcast(kB[pl.ds(off(t, n, 2), n * 64), 128 * g:128 * (g + 1)], BF16)
            s = _nn(kk, wq_of(t, g))
            tiles = [s[128 * i:128 * (i + 1)] for i in range(n)]
            tiles[-1] = jnp.where(lower, NEG, tiles[-1])
            if n == 3:
                tiles[0] = jnp.where(lower, tiles[0], NEG)
            m8 = None
            for i in range(n):
                s_ref[g * KW + 128 * i:g * KW + 128 * (i + 1)] = tiles[i]
                mc = jnp.max(tiles[i].reshape(16, 8, DP), axis=0)
                m8 = mc if m8 is None else jnp.maximum(m8, mc)
            mB_ref.at[g][...] = jnp.max(m8, axis=0, keepdims=True)

        def ex(t, g, sl):
            n = ntile(t)
            p = jnp.exp2(s_ref[g * KW:g * KW + 128 * n] - mB_ref.at[g][...]).astype(BF16)
            p_ref.at[sl][g * KW // 2:g * KW // 2 + 64 * n] = pltpu.bitcast(p, U32)

        def pv(t, g, sl):
            n = ntile(t)
            for i in range(4):
                h0 = 128 * g + HP * i
                p = pltpu.bitcast(p_ref.at[sl][g * KW // 2:g * KW // 2 + 64 * n, 128 * i:128 * (i + 1)], BF16)
                o = _nn(vB[h0:h0 + HP, pl.ds(off(t, n), n * 128)], p)
                oT[h0:h0 + HP, qsl(t)] = (o / o[DH:DH + 1, :]).astype(BF16)

        def stage(tp, te, tq, par):
            for g in range(4):
                if tp is not None:
                    pv(tp, g, 1 - par)
                if te is not None:
                    ex(te, g, par)
                if tq is not None:
                    qk(tq, g)

        stage(None, None, 0, 1)
        stage(None, 0, 1, 0)
        stage(0, 1, 2, 1)
        stage(1, 2, 3, 0)

        def body(i, carry):
            for u in range(UB):
                t = 3 + i * UB + u
                stage(t - 1, t, t + 1, (3 + u) % 2)
            return carry
        lax.fori_loop(0, 12 // UB, body, 0)
        stage(14, 15, None, 1)
        stage(15, None, None, 0)

    def loop_tok(fn):
        def body(i, c):
            fn(i)
            return c
        lax.fori_loop(0, nb, body, 0)

    loop_tok(proj_A)

    def rep_body(rep, carry):
        attn_A()

        def mid(i):
            out_proj(i, woA)
            proj_B(i)
        loop_tok(mid)
        attn_B()

        @pl.when(rep == 0)
        def _():
            def nxt(i):
                out_proj(i, woB)
                proj_A(i)
            loop_tok(nxt)

        @pl.when(rep == 1)
        def _():
            def fin(i):
                y = xT[:, tok(i)] + _nn(woB[...], oT[:, tok(i)])
                o_ref[:, tok(i)] = y.astype(BF16)
            loop_tok(fin)
        return carry

    lax.fori_loop(0, 2, rep_body, 0)


@jax.jit
def pallas_interleave_layers__grouped_kv_mqa__sliding_block__prompt_kernel(
    A_x: jax.Array,
    A_wq: jax.Array,
    A_wk: jax.Array,
    A_wv: jax.Array,
    A_wo: jax.Array,
    B_x: jax.Array,
    B_wqkv: jax.Array,
    B_wo: jax.Array,
):
    x = A_x.reshape(S, D).T
    scratch = [
        pltpu.VMEM((D, S), F32),
        pltpu.VMEM((DP + 2 * HP, D), BF16),
        pltpu.VMEM((D, DP), BF16),
        pltpu.VMEM((3 * DP, D), BF16),
        pltpu.VMEM((D, DP), BF16),
        pltpu.VMEM((DP, S), BF16),
        pltpu.VMEM((S // 2, HP), U32),
        pltpu.VMEM((HP, S), BF16),
        pltpu.VMEM((S // 2, DP), U32),
        pltpu.VMEM((DP, S), BF16),
        pltpu.VMEM((DP, S), BF16),
        pltpu.VMEM((S, NQ), F32),
        pltpu.VMEM((1, NQ), F32),
        pltpu.VMEM((2, S // 2, NQ), U32),
        pltpu.VMEM((4, 1, DP), F32),
    ]
    out = pl.pallas_call(
        _kernel,
        out_shape=jax.ShapeDtypeStruct((D, S), BF16),
        scratch_shapes=scratch,
        compiler_params=pltpu.CompilerParams(vmem_limit_bytes=100 * 1024 * 1024),
    )(x, A_wq, A_wk.T, A_wv.T, A_wo, B_wqkv, B_wo)
    return out.T.reshape(1, S, D)
```

```python
import functools
import math

import jax
import jax.numpy as jnp
from jax import lax
import jax.experimental.pallas as pl
import jax.experimental.pallas.tpu as pltpu

S = 2048
D = 448
H = 16
DH = 28
HP = 32
DP = H * HP
W = 256
EPS = 1e-5
QSCALE = (DH ** -0.5) * math.log2(math.e)
NEG = -1e30

TB = 512
SB = 256
NQ = 512
KC = 128
UA = 2
UF = 9
NPB = 3
NVB = 192
QC = 32
PK = 16
DL = 3
VL0 = NQ - 128
SAFE = 1.0 + 2.0 ** -6
L_LO = 2.0 ** -40
L_HI = 2.0 ** 20
UB = 2
KW = W + 128
SR = W + 32
F32 = jnp.float32
BF16 = jnp.bfloat16
U32 = jnp.uint32


def _nn(a, b):
    return jnp.dot(a, b, preferred_element_type=F32)


def _nt(a, b):
    return lax.dot_general(a, b, (((1,), (1,)), ((), ())), preferred_element_type=F32)


def _tn(a, b):
    return lax.dot_general(a, b, (((0,), (0,)), ((), ())), preferred_element_type=F32)


def _pad_heads(r, nheads, fill):
    parts = []
    for h in range(nheads):
        parts += [r[DH * h:DH * (h + 1)], fill]
    return jnp.concatenate(parts, axis=0)


def _wo_transpose_into(dst_ref, wo_ref):
    z = jnp.zeros((HP - DH, D), F32)
    dst_ref[...] = _pad_heads(wo_ref[...].astype(F32), H, z).astype(BF16).T


def _gate(x, dep):
    return jnp.maximum(x, jnp.minimum(dep, -jnp.inf))


def _layernorm_T(xt):
    m = jnp.sum(xt, axis=0, keepdims=True) * (1.0 / D)
    xc = xt - m
    v = jnp.sum(xc * xc, axis=0, keepdims=True) * (1.0 / D)
    return (xc * lax.rsqrt(v + EPS)).astype(BF16)


def _kernel(x_hbm, awq_hbm, awk_hbm, awv_hbm, awo_hbm, bwqkv_hbm, bwo_hbm, o_hbm,
            xin, awq_v, awk_v, awv_v, awo_v, bwqkv_v, bwo_v, ostage, sems,
            xT, wA, woA, wB, woB, qT, kA, vA, kB, vB, oT, s_ref, m_ref, p_ref, mB_ref,
            kb_ref, qb_ref, kn_ref, bad_ref, qs_ref):
    nb = S // TB

    def tok(i):
        if isinstance(i, int):
            return pl.ds(i * TB, TB)
        return pl.ds(pl.multiple_of(i * TB, TB), TB)

    def tokh(i):
        if isinstance(i, int):
            return pl.ds(i * (TB // 2), TB // 2)
        return pl.ds(pl.multiple_of(i * (TB // 2), TB // 2), TB // 2)

    w_copies = [pltpu.make_async_copy(src, dst, sems.at[k]) for k, (src, dst) in enumerate(
        [(awq_hbm, awq_v), (awk_hbm, awk_v), (awv_hbm, awv_v),
         (awo_hbm, awo_v), (bwqkv_hbm, bwqkv_v), (bwo_hbm, bwo_v)])]

    def x_copy(i):
        return pltpu.make_async_copy(x_hbm.at[:, tok(i)], xin.at[:, tok(i)], sems.at[6 + i])

    def o_copy(i):
        return pltpu.make_async_copy(ostage.at[:, tok(i)], o_hbm.at[:, tok(i)], sems.at[6 + nb + i])

    w_copies[0].start()
    w_copies[1].start()
    w_copies[2].start()
    for i in range(nb):
        x_copy(i).start()
    for cp in w_copies[3:]:
        cp.start()

    for cp in w_copies[:3]:
        cp.wait()
    wA[2 * HP:2 * HP + D, :] = awq_v[...].T
    zrow = jnp.zeros((HP - DH, D), F32)
    wA[0:2 * HP, :] = jnp.concatenate(
        [awk_v[...].astype(F32), zrow, awv_v[...].astype(F32), zrow], axis=0).astype(BF16)

    def prep_rest():
        _wo_transpose_into(woA, awo_v)
        wt = bwqkv_v[...].T
        wB[0:D, :] = wt[D:2 * D]
        wB[D:2 * D, :] = wt[0:D]
        wB[2 * D:3 * D, :] = wt[2 * D:3 * D]
        _wo_transpose_into(woB, bwo_v)

    ones_row_A = lax.broadcasted_iota(jnp.int32, (HP, NQ), 0) == DH
    zfill = jnp.zeros((HP - DH, SB), F32)
    onefill = jnp.where(lax.broadcasted_iota(jnp.int32, (HP - DH, SB), 0) == 0, 1.0, 0.0).astype(F32)
    ones_row_S = lax.broadcasted_iota(jnp.int32, (HP, SB), 0) == DH
    z3 = jnp.zeros((HP - DH - 1, SB), F32)
    nsb = TB // SB
    NVS = NVB // nsb

    def sub(i, u, n):
        if isinstance(i, int):
            return pl.ds((i * nsb + u) * n, n)
        return pl.ds(pl.multiple_of((i * nsb + u) * n, n), n)

    def proj_A(i, u, xn):
        r = _nn(wA[0:2 * HP, :], xn)
        kt = r[0:HP]
        kn_ref[...] = jnp.maximum(kn_ref[...], jnp.sum(kt * kt, axis=0, keepdims=True))
        k16 = kt.T.astype(BF16)
        kA[sub(i, u, SB // 2), :] = pltpu.bitcast(k16, U32)
        kv = k16[0:NVS].astype(F32)
        for d in range(DH):
            kb_ref.at[d][sub(i, u, NVS), :] = jnp.broadcast_to(kv[:, d:d + 1], (NVS, 128))
        vA[:, sub(i, u, SB)] = jnp.where(ones_row_S, 1.0, r[HP:2 * HP]).astype(BF16)
        q = _nn(wA[2 * HP:2 * HP + D, :], xn) * QSCALE
        parts = []
        for h in range(H):
            qh = q[DH * h:DH * (h + 1)]
            qn = jnp.sqrt(jnp.sum(qh * qh, axis=0, keepdims=True)) * SAFE
            parts += [qh, -qn, z3]
        qT[:, sub(i, u, SB)] = pltpu.bitcast(jnp.concatenate(parts, axis=0).astype(BF16), U32)

    def proj_B(i, u, xn):
        kB[sub(i, u, SB // 2), :] = pltpu.bitcast(
            _pad_heads(_nn(wB[0:D, :], xn), H, zfill).astype(BF16).T, U32)
        q = _pad_heads(_nn(wB[D:2 * D, :], xn) * QSCALE, H, zfill)
        rows = []
        for h in range(H):
            qh = q[HP * h:HP * (h + 1)]
            if h % 4:
                qh = jnp.concatenate([pltpu.roll(qh[:, 128 * t:128 * (t + 1)], 32 * (h % 4), 1)
                                      for t in range(SB // 128)], axis=1)
            rows.append(qh)
        qT[:, sub(i, u, SB)] = pltpu.bitcast(jnp.concatenate(rows, axis=0).astype(BF16), U32)
        vB[:, sub(i, u, SB)] = _pad_heads(_nn(wB[2 * D:3 * D, :], xn), H, onefill).astype(BF16)

    def out_proj(i, u, wo):
        y = xT[:, sub(i, u, SB)] + _nn(wo[...], oT[:, sub(i, u, SB)])
        xT[:, sub(i, u, SB)] = y
        return y

    def out_then_proj(i, wo, proj):
        xns = [_layernorm_T(out_proj(i, u, wo)) for u in range(nsb)]
        for u in range(nsb):
            proj(i, u, xns[u])

    nqb = S // NQ
    nblk = H * nqb
    nch = S // KC

    def blk_slices(b):
        j = b // H
        h = b % H
        if isinstance(b, int):
            return pl.ds(h * HP, HP), pl.ds(j * NQ, NQ)
        return (pl.ds(pl.multiple_of(h * HP, HP), HP), pl.ds(pl.multiple_of(j * NQ, 128), NQ))

    def load_q(b):
        j = b // H
        h = b % H
        if isinstance(b, int):
            idx = pl.ds(h * (HP // 2), HP // 2), pl.ds(j * NQ, NQ)
        else:
            idx = (pl.ds(pl.multiple_of(h * (HP // 2), HP // 2), HP // 2),
                   pl.ds(pl.multiple_of(j * NQ, 128), NQ))
        return pltpu.bitcast(qT[idx], BF16)

    def a_stage(bpv, do_ex, bqk, par):
        m_old = m_ref[...] if do_ex else None
        q = None
        if bqk is not None:
            q = jnp.where(ones_row_A, 0.0, load_q(bqk).astype(F32)).astype(BF16)
        o = None
        m8 = None
        for c in range(nch):
            rows = slice(c * KC, (c + 1) * KC)
            prow = slice(c * KC // 2, (c + 1) * KC // 2)
            if bpv is not None:
                oc = _nn(vA[:, rows], pltpu.bitcast(p_ref.at[1 - par][prow], BF16))
                o = oc if o is None else o + oc
            if do_ex:
                p = jnp.exp2(s_ref[rows] - m_old).astype(BF16)
                p_ref.at[par][prow] = pltpu.bitcast(p, U32)
            if bqk is not None:
                s = _nn(pltpu.bitcast(kA[prow], BF16), q)
                s_ref[rows] = s
                mc = jnp.max(s.reshape(KC // 8, 8, NQ), axis=0)
                m8 = mc if m8 is None else jnp.maximum(m8, mc)
        if bqk is not None:
            m_ref[...] = jnp.max(m8, axis=0, keepdims=True)
        if bpv is not None:
            oT[blk_slices(bpv)] = (o / o[DH:DH + 1, :]).astype(BF16)

    def attn_A_exact():
        npeel = (nblk - 2) % UA
        a_stage(None, False, 0, 1)
        a_stage(None, True, 1, 0)
        for b in range(1, 1 + npeel):
            a_stage(b - 1, True, b + 1, b % 2)

        def body(i, c):
            for u in range(UA):
                b = 1 + npeel + i * UA + u
                a_stage(b - 1, True, b + 1, (1 + npeel + u) % 2)
            return c
        lax.fori_loop(0, (nblk - 2 - npeel) // UA, body, 0)
        a_stage(nblk - 2, True, None, (nblk - 1) % 2)
        a_stage(nblk - 1, False, None, nblk % 2)

    narrow, wide = [], []
    for j in range(S // SB):
        narrow += [(r, r + QC, VL0) for r in range(j * SB, j * SB + NVS, QC)]
        wide += [(r, r + QC, NQ) for r in range(j * SB + NVS, (j + 1) * SB, QC)]
    chunks = []
    ni = wi = 0
    while ni < len(narrow) or wi < len(wide):
        if (ni * len(wide) <= wi * len(narrow) and ni < len(narrow)) or wi >= len(wide):
            chunks.append(narrow[ni])
            ni += 1
        else:
            chunks.append(wide[wi])
            wi += 1
    n_it = len(chunks)
    pieces = [(j * NVS + k0, j * SB + k0) for j in range(S // SB) for k0 in range(0, NVS, PK)]
    npieces = len(pieces)

    def f_stage(bpv, bqk, par, kmax):
        pw = p_ref.at[par]
        prd = p_ref.at[(par + NPB - 1) % NPB]
        qbr = qb_ref.at[par]
        q = None
        if bqk is not None:
            q = load_q(bqk)
            qsr = qs_ref.at[par]
            qsr[...] = pltpu.bitcast(q, U32)
            qf = q[:, VL0:].astype(F32)
            for d in range(DH):
                qbr[d * 8:(d + 1) * 8, :] = jnp.broadcast_to(qf[d:d + 1, :], (8, 128))
            qbr[DH * 8:(DH + 1) * 8, :] = jnp.broadcast_to(qf[DH:DH + 1, :] * kmax, (8, 128))
        o = None
        pv_done = 0
        pending = {}
        for it, (r0, r1, nc) in enumerate(chunks):
            if bpv is not None:
                while pv_done < nch and pv_done * n_it // nch <= it:
                    c = pv_done
                    oc = _nn(vA[:, c * KC:(c + 1) * KC],
                             pltpu.bitcast(prd[c * KC // 2:(c + 1) * KC // 2], BF16))
                    o = oc if o is None else o + oc
                    pv_done += 1
            if bqk is None:
                continue
            s = _nn(pltpu.bitcast(kA[r0 // 2:r1 // 2], BF16), pltpu.bitcast(qsr[:, 0:nc], BF16))
            if it in pending:
                top = s[0:8, 0:128]
                for dep in pending.pop(it):
                    top = _gate(top, dep)
                row0 = jnp.concatenate([top, s[0:8, 128:nc]], axis=1)
                s = jnp.concatenate([row0, s[8:]], axis=0)
            pw[r0 // 2:r1 // 2, 0:nc] = pltpu.bitcast(jnp.exp2(s).astype(BF16), U32)
            for pi, (kb0, k0) in enumerate(pieces):
                if 1 + pi * (n_it - 2) // npieces != it:
                    continue
                init = jnp.concatenate([qbr[DH * 8:(DH + 1) * 8, :]] * (PK // 8), axis=0)
                dep = jnp.concatenate([s[0:8, 128:256]] * (PK // 8), axis=0)
                acc = _gate(init, dep)
                for d in range(DH):
                    kb = kb_ref.at[d][kb0:kb0 + PK, :]
                    qrow = jnp.concatenate([qbr[d * 8:(d + 1) * 8, :]] * (PK // 8), axis=0)
                    acc = acc + kb * qrow
                pw[k0 // 2:(k0 + PK) // 2, VL0:] = pltpu.bitcast(jnp.exp2(acc).astype(BF16), U32)
                if it + DL < n_it:
                    pending.setdefault(it + DL, []).append(acc[PK - 8:PK])
        if bpv is not None:
            l = o[DH:DH + 1, :]
            ok = jnp.logical_and(l >= L_LO, l <= L_HI)
            bad_ref[...] = jnp.maximum(bad_ref[...], jnp.where(ok, 0, 1))
            oT[blk_slices(bpv)] = (o / l).astype(BF16)

    def set_k_col(val):
        lane = lax.broadcasted_iota(jnp.int32, (S, HP), 1)
        k = pltpu.bitcast(kA[...], BF16).astype(F32)
        kA[...] = pltpu.bitcast(jnp.where(lane == DH, val, k).astype(BF16), U32)

    def attn_A():
        kmax = jnp.sqrt(jnp.max(kn_ref[...], axis=1, keepdims=True)) * SAFE
        kmax = kmax.astype(BF16).astype(F32)
        set_k_col(kmax)
        bad_ref[...] = jnp.zeros((1, NQ), jnp.int32)
        npeel = (nblk - 1) % UF
        f_stage(None, 0, 0, kmax)
        for b in range(1, 1 + npeel):
            f_stage(b - 1, b, b % NPB, kmax)

        def body(i, c):
            for u in range(UF):
                b = 1 + npeel + i * UF + u
                f_stage(b - 1, b, (1 + npeel + u) % NPB, kmax)
            return c
        lax.fori_loop(0, (nblk - 1 - npeel) // UF, body, 0)
        f_stage(nblk - 1, None, nblk % NPB, kmax)

        @pl.when(jnp.max(bad_ref[...]) > 0)
        def _():
            set_k_col(0.0)
            attn_A_exact()

    def attn_B():
        r = lax.broadcasted_iota(jnp.int32, (32, 128), 0)
        c = lax.broadcasted_iota(jnp.int32, (32, 128), 1) & 31
        lower = r > c
        lq16 = lax.broadcasted_iota(jnp.int32, (16, 128), 1) >> 5
        lq8 = lax.broadcasted_iota(jnp.int32, (8, 128), 1) >> 5
        zq = jnp.zeros((16, 128), U32)
        z8 = jnp.zeros((8, 128), U32)

        def qsl(t):
            return pl.ds(t * 128, 128) if isinstance(t, int) else pl.ds(pl.multiple_of(t * 128, 128), 128)

        def win(t, b):
            if isinstance(t, int):
                skip = max(0, W - 128 * t - 32 * b)
                return skip, SR - skip
            return 0, SR

        def ntile(t):
            return min(t + 1, 3) if isinstance(t, int) else 3

        def qk(t, g):
            qg = qT[64 * g:64 * (g + 1), qsl(t)]
            for b in range(4):
                wb = jnp.concatenate([jnp.where(lq16 == (b + i) % 4, qg[16 * i:16 * (i + 1)], zq)
                                      for i in range(4)], axis=0)
                skip, n = win(t, b)
                if isinstance(t, int):
                    ks = pl.ds((128 * t + 32 * b - W + skip) // 2, n // 2)
                else:
                    ks = pl.ds(pl.multiple_of(64 * t + 16 * b - W // 2, 16), n // 2)
                s = _nn(pltpu.bitcast(kB[ks, 128 * g:128 * (g + 1)], BF16), pltpu.bitcast(wb, BF16))
                parts = []
                if skip == 0:
                    parts.append(jnp.where(lower, s[0:32], NEG))
                    parts.append(s[32:n - 32])
                elif n > 32:
                    parts.append(s[0:n - 32])
                parts.append(jnp.where(lower, NEG, s[n - 32:n]))
                s = jnp.concatenate(parts, axis=0)
                s_ref[g * SR + skip:(g + 1) * SR, 128 * b:128 * (b + 1)] = s
                m8 = jnp.max(s.reshape(n // 8, 8, 128), axis=0)
                mB_ref.at[g][:, 128 * b:128 * (b + 1)] = jnp.max(m8, axis=0, keepdims=True)

        def ex(t, g, sl):
            n3 = ntile(t)
            pb = g * KW // 2
            ps = []
            for b in range(4):
                skip, n = win(t, b)
                m = mB_ref.at[g][:, 128 * b:128 * (b + 1)]
                p = jnp.exp2(s_ref[g * SR + skip:(g + 1) * SR, 128 * b:128 * (b + 1)] - m).astype(BF16)
                ps.append((pltpu.bitcast(p, U32), skip))
            for i in range(4):
                rows = []
                for j in range((3 - n3) * 8, 24):
                    out = None
                    for b in range(4):
                        pk, skip = ps[b]
                        jj = j - 2 * b - skip // 16
                        src = pk[8 * jj:8 * (jj + 1)] if 0 <= jj < (SR - skip) // 16 else z8
                        out = src if out is None else jnp.where(lq8 == (b + i) % 4, src, out)
                    rows.append(out)
                p_ref.at[sl][pb:pb + 64 * n3, 128 * i:128 * (i + 1)] = jnp.concatenate(rows, axis=0)

        def pv(t, g, sl):
            n = ntile(t)
            pb = g * KW // 2
            if isinstance(t, int):
                ks = pl.ds((t + 1 - n) * 128, n * 128)
            else:
                ks = pl.ds(pl.multiple_of((t - 2) * 128, 128), n * 128)
            for i in range(4):
                h0 = 128 * g + HP * i
                p = pltpu.bitcast(p_ref.at[sl][pb:pb + 64 * n, 128 * i:128 * (i + 1)], BF16)
                o = _nn(vB[h0:h0 + HP, ks], p)
                o = o / o[DH:DH + 1, :]
                if i:
                    o = pltpu.roll(o, 128 - 32 * i, 1)
                oT[h0:h0 + HP, qsl(t)] = o.astype(BF16)

        def stage(tp, te, tq, par):
            for g in range(4):
                if tp is not None:
                    pv(tp, g, 1 - par)
                if te is not None:
                    ex(te, g, par)
                if tq is not None:
                    qk(tq, g)

        stage(None, None, 0, 1)
        stage(None, 0, 1, 0)
        stage(0, 1, 2, 1)
        stage(1, 2, 3, 0)

        def body(i, carry):
            for u in range(UB):
                t = 3 + i * UB + u
                stage(t - 1, t, t + 1, (3 + u) % 2)
            return carry
        lax.fori_loop(0, 12 // UB, body, 0)
        stage(14, 15, None, 1)
        stage(15, None, None, 0)

    def loop_tok(fn):
        def body(i, c):
            fn(i)
            return c
        lax.fori_loop(0, nb, body, 0)

    kn_ref[...] = jnp.zeros((1, SB), F32)

    def first(i):
        x_copy(i).wait()
        for u in range(nsb):
            xt = xin[:, sub(i, u, SB)].astype(F32)
            xT[:, sub(i, u, SB)] = xt
            proj_A(i, u, _layernorm_T(xt))
    loop_tok(first)

    for cp in w_copies[3:]:
        cp.wait()

    def rep_body(rep, carry):
        prep_rest()
        attn_A()
        loop_tok(lambda i: out_then_proj(i, woA, proj_B))
        attn_B()

        @pl.when(rep == 0)
        def _():
            kn_ref[...] = jnp.zeros((1, SB), F32)
            loop_tok(lambda i: out_then_proj(i, woB, proj_A))

        @pl.when(rep == 1)
        def _():
            def fin(i):
                y = xT[:, tok(i)] + _nn(woB[...], oT[:, tok(i)])
                ostage[:, tok(i)] = y.astype(BF16)
                o_copy(i).start()
            loop_tok(fin)
        return carry

    lax.fori_loop(0, 2, rep_body, 0)
    for i in range(nb):
        o_copy(i).wait()


@jax.jit
def pallas_interleave_layers__grouped_kv_mqa__sliding_block__prompt_kernel(
    A_x: jax.Array,
    A_wq: jax.Array,
    A_wk: jax.Array,
    A_wv: jax.Array,
    A_wo: jax.Array,
    B_x: jax.Array,
    B_wqkv: jax.Array,
    B_wo: jax.Array,
):
    x = A_x.reshape(S, D).T
    scratch = [
        pltpu.VMEM((D, S), BF16),
        pltpu.VMEM((D, D), BF16),
        pltpu.VMEM((DH, D), BF16),
        pltpu.VMEM((DH, D), BF16),
        pltpu.VMEM((D, D), BF16),
        pltpu.VMEM((D, 3 * D), BF16),
        pltpu.VMEM((D, D), BF16),
        pltpu.VMEM((D, S), BF16),
        pltpu.SemaphoreType.DMA((6 + 2 * (S // TB),)),
        pltpu.VMEM((D, S), F32),
        pltpu.VMEM((D + 2 * HP, D), BF16),
        pltpu.VMEM((D, DP), BF16),
        pltpu.VMEM((3 * D, D), BF16),
        pltpu.VMEM((D, DP), BF16),
        pltpu.VMEM((DP // 2, S), U32),
        pltpu.VMEM((S // 2, HP), U32),
        pltpu.VMEM((HP, S), BF16),
        pltpu.VMEM((S // 2, DP), U32),
        pltpu.VMEM((DP, S), BF16),
        pltpu.VMEM((DP, S), BF16),
        pltpu.VMEM((S, NQ), F32),
        pltpu.VMEM((1, NQ), F32),
        pltpu.VMEM((NPB, S // 2, NQ), U32),
        pltpu.VMEM((4, 1, DP), F32),
        pltpu.VMEM((DH, (S // TB) * NVB, 128), F32),
        pltpu.VMEM((NPB, (DH + 1) * 8, 128), F32),
        pltpu.VMEM((1, SB), F32),
        pltpu.VMEM((1, NQ), jnp.int32),
        pltpu.VMEM((NPB, HP // 2, NQ), U32),
    ]
    out = pl.pallas_call(
        _kernel,
        out_shape=jax.ShapeDtypeStruct((D, S), BF16),
        in_specs=[pl.BlockSpec(memory_space=pl.ANY)] * 7,
        out_specs=pl.BlockSpec(memory_space=pl.ANY),
        scratch_shapes=scratch,
        compiler_params=pltpu.CompilerParams(vmem_limit_bytes=100 * 1024 * 1024),
    )(x, A_wq, A_wk.T, A_wv.T, A_wo, B_wqkv, B_wo)
    return out.T.reshape(1, S, D)
```

```python
import math

import jax
import jax.numpy as jnp
from jax import lax
import jax.experimental.pallas as pl
import jax.experimental.pallas.tpu as pltpu

S = 2048
D = 448
H = 16
DH = 28
HP = 32
DP = H * HP
W = 256
EPS = 1e-5
QSCALE = (DH ** -0.5) * math.log2(math.e)
NEG = -1e30

TB = 512
SB = 256
NQ = 512
KC = 128
UF = 9
NPB = 3
PVS = 1
SPLIT = 3
NVB = 192
QC = 32
PK = 16
DL = 2
VL0 = NQ - 128
SAFE = 1.0 + 2.0 ** -6
L_LO = 2.0 ** -40
L_HI = 2.0 ** 20
UB = 4
SR = W + 32
F32 = jnp.float32
BF16 = jnp.bfloat16
U32 = jnp.uint32


def _nn(a, b):
    return jnp.dot(a, b, preferred_element_type=F32)


def _pad_heads(r, nheads, fill):
    parts = []
    for h in range(nheads):
        parts += [r[DH * h:DH * (h + 1)], fill]
    return jnp.concatenate(parts, axis=0)


def _wo_transpose_into(dst_ref, wo_ref):
    z = jnp.zeros((HP - DH, D), F32)
    dst_ref[...] = _pad_heads(wo_ref[...].astype(F32), H, z).astype(BF16).T


def _gate(x, dep):
    return jnp.maximum(x, jnp.minimum(dep, -jnp.inf))


def _layernorm_T(xt):
    m = jnp.sum(xt, axis=0, keepdims=True) * (1.0 / D)
    xc = xt - m
    v = jnp.sum(xc * xc, axis=0, keepdims=True) * (1.0 / D)
    return (xc * lax.rsqrt(v + EPS)).astype(BF16)


def _kernel(x_hbm, awq_hbm, awk_hbm, awv_hbm, awo_hbm, bwqkv_hbm, bwo_hbm, o_hbm,
            xin, awq_v, awk_v, awv_v, awo_v, bwqkv_v, bwo_v, ostage, sems,
            xT, wA, woA, wB, woB, qT, kA, vA, kB, vB, oT, s_ref, p_ref, mB_ref,
            kb_ref, qb_ref, kn_ref, bad_ref, qs_ref):
    nb = S // TB

    def tok(i):
        if isinstance(i, int):
            return pl.ds(i * TB, TB)
        return pl.ds(pl.multiple_of(i * TB, TB), TB)

    w_copies = [pltpu.make_async_copy(src, dst, sems.at[k]) for k, (src, dst) in enumerate(
        [(awq_hbm, awq_v), (awk_hbm, awk_v), (awv_hbm, awv_v),
         (awo_hbm, awo_v), (bwqkv_hbm, bwqkv_v), (bwo_hbm, bwo_v)])]

    def x_copy(i):
        return pltpu.make_async_copy(x_hbm.at[:, tok(i)], xin.at[:, tok(i)], sems.at[6 + i])

    def o_copy(j):
        cols = pl.ds(j * SB, SB) if isinstance(j, int) else pl.ds(pl.multiple_of(j * SB, SB), SB)
        return pltpu.make_async_copy(ostage.at[:, cols], o_hbm.at[:, cols], sems.at[6 + nb + j])

    w_copies[0].start()
    w_copies[1].start()
    w_copies[2].start()
    for i in range(nb):
        x_copy(i).start()
    for cp in w_copies[3:]:
        cp.start()

    for cp in w_copies[:3]:
        cp.wait()
    wA[2 * HP:2 * HP + D, :] = awq_v[...].T
    zrow = jnp.zeros((HP - DH, D), F32)
    wA[0:2 * HP, :] = jnp.concatenate(
        [awk_v[...].astype(F32), zrow, awv_v[...].astype(F32), zrow], axis=0).astype(BF16)

    def prep_rest():
        _wo_transpose_into(woA, awo_v)
        wt = bwqkv_v[...].T
        wB[0:D, :] = wt[D:2 * D]
        wB[D:2 * D, :] = wt[0:D]
        wB[2 * D:3 * D, :] = wt[2 * D:3 * D]
        _wo_transpose_into(woB, bwo_v)

    ones_row_A = lax.broadcasted_iota(jnp.int32, (HP, NQ), 0) == DH
    zfill = jnp.zeros((HP - DH, SB), F32)
    onefill = jnp.where(lax.broadcasted_iota(jnp.int32, (HP - DH, SB), 0) == 0, 1.0, 0.0).astype(F32)
    ones_row_S = lax.broadcasted_iota(jnp.int32, (HP, SB), 0) == DH
    z3 = jnp.zeros((HP - DH - 1, SB), F32)
    nsb = TB // SB
    NVS0 = -(-NVB // 32) * 16
    NVSL = [NVS0, NVB - NVS0]

    def sub(i, u, n):
        if isinstance(i, int):
            return pl.ds((i * nsb + u) * n, n)
        return pl.ds(pl.multiple_of((i * nsb + u) * n, n), n)

    def proj_A(i, u, xn):
        r = _nn(wA[0:2 * HP, :], xn)
        kt = r[0:HP]
        kn = jnp.max(jnp.sum(kt * kt, axis=0, keepdims=True), axis=1, keepdims=True)
        kn_ref[...] = jnp.maximum(kn_ref[...], kn)
        k16 = kt.T.astype(BF16)
        kA[sub(i, u, SB // 2), :] = pltpu.bitcast(k16, U32)
        nv = NVSL[u]
        kv = k16[0:nv].astype(F32)
        v0 = i * NVB + u * NVS0
        vrows = pl.ds(v0, nv) if isinstance(i, int) else pl.ds(pl.multiple_of(v0, 16), nv)
        for d in range(DH):
            kb_ref.at[d][vrows, :] = jnp.broadcast_to(kv[:, d:d + 1], (nv, 128))
        vA[:, sub(i, u, SB)] = jnp.where(ones_row_S, 1.0, r[HP:2 * HP]).astype(BF16)

    def proj_A2(i, u, xn):
        q = _nn(wA[2 * HP:2 * HP + D, :], xn) * QSCALE
        parts = []
        for h in range(H):
            qh = q[DH * h:DH * (h + 1)]
            qn = jnp.sqrt(jnp.sum(qh * qh, axis=0, keepdims=True)) * SAFE
            parts += [qh, -qn, z3]
        qT[:, sub(i, u, SB)] = pltpu.bitcast(jnp.concatenate(parts, axis=0).astype(BF16), U32)

    def proj_B(i, u, xn):
        kB[sub(i, u, SB // 2), :] = pltpu.bitcast(
            _pad_heads(_nn(wB[0:D, :], xn), H, zfill).astype(BF16).T, U32)
        q = _pad_heads(_nn(wB[D:2 * D, :], xn) * QSCALE, H, zfill)
        rows = []
        for h in range(H):
            qh = q[HP * h:HP * (h + 1)]
            if h % 4:
                qh = jnp.concatenate([pltpu.roll(qh[:, 128 * t:128 * (t + 1)], 32 * (h % 4), 1)
                                      for t in range(SB // 128)], axis=1)
            rows.append(qh)
        qT[:, sub(i, u, SB)] = pltpu.bitcast(jnp.concatenate(rows, axis=0).astype(BF16), U32)
        vB[:, sub(i, u, SB)] = _pad_heads(_nn(wB[2 * D:3 * D, :], xn), H, onefill).astype(BF16)

    def out_proj(i, u, wo):
        y = xT[:, sub(i, u, SB)] + _nn(wo[...], oT[:, sub(i, u, SB)])
        xT[:, sub(i, u, SB)] = y
        return y

    def out_then_proj(i, wo, *projs):
        xns = [_layernorm_T(out_proj(i, u, wo)) for u in range(nsb)]
        for u in range(nsb):
            for proj in projs:
                proj(i, u, xns[u])

    nqb = S // NQ
    nblk = H * nqb
    nch = S // KC

    def blk_slices(b):
        j = b // H
        h = b % H
        if isinstance(b, int):
            return pl.ds(h * HP, HP), pl.ds(j * NQ, NQ)
        return (pl.ds(pl.multiple_of(h * HP, HP), HP), pl.ds(pl.multiple_of(j * NQ, 128), NQ))

    def load_q(b):
        j = b // H
        h = b % H
        if isinstance(b, int):
            idx = pl.ds(h * (HP // 2), HP // 2), pl.ds(j * NQ, NQ)
        else:
            idx = (pl.ds(pl.multiple_of(h * (HP // 2), HP // 2), HP // 2),
                   pl.ds(pl.multiple_of(j * NQ, 128), NQ))
        return pltpu.bitcast(qT[idx], BF16)

    def attn_A_exact():
        KE = 256

        def blk(b, carry):
            q = jnp.where(ones_row_A, 0.0, load_q(b).astype(F32)).astype(BF16)

            def pass1(c, m8):
                s = _nn(pltpu.bitcast(kA[pl.ds(pl.multiple_of(c * (KE // 2), KE // 2), KE // 2), :], BF16), q)
                s_ref[pl.ds(pl.multiple_of(c * KE, KE), KE), :] = s
                return jnp.maximum(m8, jnp.max(s.reshape(KE // 8, 8, NQ), axis=0))
            m8 = lax.fori_loop(0, S // KE, pass1, jnp.full((8, NQ), -jnp.inf, F32))
            m = jnp.max(m8, axis=0, keepdims=True)

            def pass2(c, o):
                rows = pl.ds(pl.multiple_of(c * KE, KE), KE)
                p = jnp.exp2(s_ref[rows, :] - m).astype(BF16)
                return o + _nn(vA[:, rows], p)
            o = lax.fori_loop(0, S // KE, pass2, jnp.zeros((HP, NQ), F32))
            oT[blk_slices(b)] = (o / o[DH:DH + 1, :]).astype(BF16)
            return carry
        lax.fori_loop(0, nblk, blk, 0)

    narrow, wide = [], []
    for j in range(S // SB):
        NVS = NVSL[j % nsb]
        narrow += [(r, min(r + QC, j * SB + NVS), VL0) for r in range(j * SB, j * SB + NVS, QC)]
        wide += [(r, min(r + QC, (j + 1) * SB), NQ) for r in range(j * SB + NVS, (j + 1) * SB, QC)]
    chunks = []
    ni = wi = 0
    while ni < len(narrow) or wi < len(wide):
        if (ni * len(wide) <= wi * len(narrow) and ni < len(narrow)) or wi >= len(wide):
            chunks.append(narrow[ni])
            ni += 1
        else:
            chunks.append(wide[wi])
            wi += 1
    n_it = len(chunks)
    pieces = [((j // nsb) * NVB + (j % nsb) * NVS0 + k0, j * SB + k0)
              for j in range(S // SB) for k0 in range(0, NVSL[j % nsb], PK)]
    npieces = len(pieces)

    def f_first(par):
        qsr = qs_ref.at[par]
        qsr[...] = pltpu.bitcast(load_q(0), U32)
        for c in range(nch):
            s = _nn(pltpu.bitcast(kA[c * KC // 2:(c + 1) * KC // 2], BF16), pltpu.bitcast(qsr[...], BF16))
            p_ref.at[par][c * KC // 2:(c + 1) * KC // 2] = pltpu.bitcast(jnp.exp2(s).astype(BF16), U32)

    per, kk, ww = nch // PVS, KC * PVS, NQ // PVS

    def f_stage(bpv, bqk, par, kmax):
        pw = p_ref.at[par]
        prd = p_ref.at[(par + NPB - 1) % NPB]
        qbr = qb_ref.at[par]
        q = None
        if bqk is not None:
            q = load_q(bqk)
            qsr = qs_ref.at[par]
            qsr[...] = pltpu.bitcast(q, U32)
            qf = q[:, VL0:].astype(F32)
            for d in range(DH):
                qbr[d * 8:(d + 1) * 8, :] = jnp.broadcast_to(qf[d:d + 1, :], (8, 128))
            qbr[DH * 8:(DH + 1) * 8, :] = jnp.broadcast_to(qf[DH:DH + 1, :] * kmax, (8, 128))
        o = None
        pv_done = 0
        pending = {}
        carry_over = []
        for it, (r0, r1, nc) in enumerate(chunks):
            if bpv is not None:
                while pv_done < nch and pv_done * n_it // nch <= it:
                    hf, cc = pv_done // per, pv_done % per
                    oc = _nn(vA[:, cc * kk:(cc + 1) * kk],
                             pltpu.bitcast(prd[cc * kk // 2:(cc + 1) * kk // 2, hf * ww:(hf + 1) * ww], BF16))
                    o = oc if cc == 0 else o + oc
                    if cc == per - 1:
                        l = o[DH:DH + 1, :]
                        ok = jnp.logical_and(l >= L_LO, l <= L_HI)
                        bad_ref[:, hf * ww:(hf + 1) * ww] = jnp.maximum(
                            bad_ref[:, hf * ww:(hf + 1) * ww], jnp.where(ok, 0.0, 1.0))
                        rs_, cs_ = blk_slices(bpv)
                        st = cs_.start + hf * ww
                        cols = pl.ds(st if isinstance(st, int) else pl.multiple_of(st, 128), ww)
                        oT[rs_, cols] = (o / l).astype(BF16)
                    pv_done += 1
            if bqk is None:
                continue
            s = _nn(pltpu.bitcast(kA[r0 // 2:r1 // 2], BF16), pltpu.bitcast(qsr[:, 0:nc], BF16))
            if it in pending:
                top = s[0:8, 0:128]
                for dep in pending.pop(it):
                    top = _gate(top, dep)
                row0 = jnp.concatenate([top, s[0:8, 128:nc]], axis=1)
                s = jnp.concatenate([row0, s[8:]], axis=0)
            pw[r0 // 2:r1 // 2, 0:nc] = pltpu.bitcast(jnp.exp2(s).astype(BF16), U32)
            dep = jnp.concatenate([s[0:8, 128:256]] * (PK // 8), axis=0)
            work = carry_over
            carry_over = []
            for pi, (kb0, k0) in enumerate(pieces):
                if 1 + pi * (n_it - 1 - SPLIT) // npieces == it:
                    init = jnp.concatenate([qbr[DH * 8:(DH + 1) * 8, :]] * (PK // 8), axis=0)
                    work.append((kb0, k0, 0, init))
            for kb0, k0, part, acc in work:
                acc = _gate(acc, dep)
                d0, d1 = part * DH // SPLIT, (part + 1) * DH // SPLIT
                kb = kb_ref[d0:d1, kb0:kb0 + PK, :]
                qr = qbr[d0 * 8:d1 * 8, :].reshape(d1 - d0, 8, 128)
                prod = kb * jnp.concatenate([qr] * (PK // 8), axis=1)
                acc = jnp.sum(jnp.concatenate([acc[None], prod], axis=0), axis=0)
                if part + 1 < SPLIT:
                    carry_over.append((kb0, k0, part + 1, acc))
                    continue
                pw[k0 // 2:(k0 + PK) // 2, VL0:] = pltpu.bitcast(jnp.exp2(acc).astype(BF16), U32)
                if it + DL < n_it:
                    pending.setdefault(it + DL, []).append(acc[PK - 8:PK])
        assert not carry_over

    def set_k_col(val):
        lane = lax.broadcasted_iota(jnp.int32, (S, HP), 1)
        k = pltpu.bitcast(kA[...], BF16).astype(F32)
        kA[...] = pltpu.bitcast(jnp.where(lane == DH, val, k).astype(BF16), U32)

    def attn_A():
        kmax = jnp.sqrt(kn_ref[...]) * SAFE
        kmax = kmax.astype(BF16).astype(F32)
        set_k_col(kmax[:, 0:HP])
        bad_ref[...] = jnp.zeros((1, NQ), F32)
        f_first(0)

        def body(i, c):
            for u in range(NPB):
                b = 1 + i * NPB + u
                f_stage(b - 1, b, (1 + u) % NPB, kmax)
            return c
        lax.fori_loop(0, (nblk - 1) // NPB, body, 0, unroll=UF // NPB)
        f_stage(nblk - 1, None, nblk % NPB, kmax)

        @pl.when(jnp.max(bad_ref[...]) > 0.5)
        def _():
            set_k_col(0.0)
            attn_A_exact()

    def attn_B():
        r = lax.broadcasted_iota(jnp.int32, (32, 128), 0)
        c = lax.broadcasted_iota(jnp.int32, (32, 128), 1) & 31
        lower = r > c
        lq16 = lax.broadcasted_iota(jnp.int32, (16, 128), 1) >> 5
        lq8 = lax.broadcasted_iota(jnp.int32, (64, 128), 1) >> 5
        zq = jnp.zeros((16, 128), U32)

        def qsl(t):
            return pl.ds(t * 128, 128) if isinstance(t, int) else pl.ds(pl.multiple_of(t * 128, 128), 128)

        def win(t, b):
            if isinstance(t, int):
                skip = max(0, W - 128 * t - 32 * b)
                return skip, SR - skip
            return 0, SR

        def ntile(t):
            return min(t + 1, 3) if isinstance(t, int) else 3

        def qk(t, g):
            qg = qT[64 * g:64 * (g + 1), qsl(t)]
            for b in range(4):
                wb = jnp.concatenate([jnp.where(lq16 == (b + i) % 4, qg[16 * i:16 * (i + 1)], zq)
                                      for i in range(4)], axis=0)
                skip, n = win(t, b)
                if isinstance(t, int):
                    ks = pl.ds((128 * t + 32 * b - W + skip) // 2, n // 2)
                else:
                    ks = pl.ds(pl.multiple_of(64 * t + 16 * b - W // 2, 16), n // 2)
                s = _nn(pltpu.bitcast(kB[ks, 128 * g:128 * (g + 1)], BF16), pltpu.bitcast(wb, BF16))
                parts = []
                if skip == 0:
                    parts.append(jnp.where(lower, s[0:32], NEG))
                    parts.append(s[32:n - 32])
                elif n > 32:
                    parts.append(s[0:n - 32])
                parts.append(jnp.where(lower, NEG, s[n - 32:n]))
                s = jnp.concatenate(parts, axis=0)
                s_ref[g * SR + skip:(g + 1) * SR, 128 * b:128 * (b + 1)] = s
                m8 = jnp.max(s.reshape(n // 8, 8, 128), axis=0)
                mB_ref.at[g][:, 128 * b:128 * (b + 1)] = jnp.max(m8, axis=0, keepdims=True)

        podd = (lq8 & 1) == 1
        plo = lq8 < 2

        def ex(t, g, sl):
            pr = p_ref.at[sl]
            pb = g * SR // 2
            if isinstance(t, int) and t < 2:
                for b in range(4):
                    skip, n = win(t, b)
                    m = mB_ref.at[g][:, 128 * b:128 * (b + 1)]
                    p = jnp.exp2(s_ref[g * SR + skip:(g + 1) * SR, 128 * b:128 * (b + 1)] - m).astype(BF16)
                    pr[pb + skip // 2:pb + SR // 2, 128 * b:128 * (b + 1)] = pltpu.bitcast(p, U32)
            else:
                p = jnp.exp2(s_ref[g * SR:(g + 1) * SR, :] - mB_ref.at[g][...]).astype(BF16)
                pr[pb:pb + SR // 2, :] = pltpu.bitcast(p, U32)

        def pv(t, g, sl):
            n = ntile(t)
            pr = p_ref.at[sl]
            pb = g * SR // 2
            os_ = [None] * 4
            for kt in range(3 - n, 3):
                if isinstance(t, int):
                    ks = pl.ds((t - 2 + kt) * 128, 128)
                else:
                    ks = pl.ds(pl.multiple_of((t - 2 + kt) * 128, 128), 128)
                a = []
                for b in range(4):
                    skip, _ = win(t, b)
                    lo = max(8 * kt - 2 * b, skip // 16)
                    hi = min(8 * kt - 2 * b + 8, SR // 16)
                    parts = []
                    if lo > 8 * kt - 2 * b:
                        parts.append(jnp.zeros((8 * (min(lo, 8 * kt - 2 * b + 8) - (8 * kt - 2 * b)), 128), U32))
                    if hi > lo:
                        parts.append(pr[pb + 8 * lo:pb + 8 * hi, 128 * b:128 * (b + 1)])
                        if hi < 8 * kt - 2 * b + 8:
                            parts.append(jnp.zeros((8 * (8 * kt - 2 * b + 8 - hi), 128), U32))
                    a.append(parts[0] if len(parts) == 1 else jnp.concatenate(parts, axis=0))
                e0, e1 = jnp.where(podd, a[1], a[0]), jnp.where(podd, a[3], a[2])
                o0, o1 = jnp.where(podd, a[0], a[3]), jnp.where(podd, a[2], a[1])
                outs = [jnp.where(plo, e0, e1), jnp.where(plo, o0, o1),
                        jnp.where(plo, e1, e0), jnp.where(plo, o1, o0)]
                for i in range(4):
                    h0 = 128 * g + HP * i
                    p = pltpu.bitcast(outs[i], BF16)
                    oc = _nn(vB[h0:h0 + HP, ks], p)
                    os_[i] = oc if os_[i] is None else os_[i] + oc
            for i in range(4):
                h0 = 128 * g + HP * i
                o = os_[i] / os_[i][DH:DH + 1, :]
                if i:
                    o = pltpu.roll(o, 128 - 32 * i, 1)
                oT[h0:h0 + HP, qsl(t)] = o.astype(BF16)

        def stage(tp, te, tq, par):
            for g in range(4):
                if tp is not None:
                    pv(tp, g, 1 - par)
                if te is not None:
                    ex(te, g, par)
                if tq is not None:
                    qk(tq, g)

        stage(None, None, 0, 1)
        stage(None, 0, 1, 0)
        stage(0, 1, 2, 1)
        stage(1, 2, 3, 0)

        def body(i, carry):
            for u in range(2):
                t = 3 + i * 2 + u
                stage(t - 1, t, t + 1, (3 + u) % 2)
            return carry
        lax.fori_loop(0, 6, body, 0, unroll=UB // 2)
        stage(14, 15, None, 1)
        stage(15, None, None, 0)

    def loop_tok(fn, unroll=1):
        def body(i, c):
            fn(i)
            return c
        lax.fori_loop(0, nb, body, 0, unroll=unroll)

    kn_ref[...] = jnp.zeros((1, 128), F32)

    def first(i):
        x_copy(i).wait()
        xns = []
        for u in range(nsb):
            xt = xin[:, sub(i, u, SB)].astype(F32)
            xT[:, sub(i, u, SB)] = xt
            xns.append(_layernorm_T(xt))
        for proj in (proj_A, proj_A2):
            for u in range(nsb):
                proj(i, u, xns[u])
    loop_tok(first)

    for cp in w_copies[3:]:
        cp.wait()

    def rep_body(rep, carry):
        prep_rest()
        attn_A()

        loop_tok(lambda i: out_then_proj(i, woA, proj_B), unroll=2)
        attn_B()

        @pl.when(rep == 0)
        def _():
            kn_ref[...] = jnp.zeros((1, 128), F32)
            loop_tok(lambda i: out_then_proj(i, woB, proj_A, proj_A2))

        @pl.when(rep == 1)
        def _():
            def fin(i):
                for u in range(nsb):
                    y = xT[:, sub(i, u, SB)] + _nn(woB[...], oT[:, sub(i, u, SB)])
                    ostage[:, sub(i, u, SB)] = y.astype(BF16)
                    o_copy(i * nsb + u).start()
            loop_tok(fin)
        return carry

    lax.fori_loop(0, 2, rep_body, 0)
    for j in range(S // SB):
        o_copy(j).wait()


@jax.jit
def pallas_interleave_layers__grouped_kv_mqa__sliding_block__prompt_kernel(
    A_x: jax.Array,
    A_wq: jax.Array,
    A_wk: jax.Array,
    A_wv: jax.Array,
    A_wo: jax.Array,
    B_x: jax.Array,
    B_wqkv: jax.Array,
    B_wo: jax.Array,
):
    x = A_x.reshape(S, D).T
    scratch = [
        pltpu.VMEM((D, S), BF16),
        pltpu.VMEM((D, D), BF16),
        pltpu.VMEM((DH, D), BF16),
        pltpu.VMEM((DH, D), BF16),
        pltpu.VMEM((D, D), BF16),
        pltpu.VMEM((D, 3 * D), BF16),
        pltpu.VMEM((D, D), BF16),
        pltpu.VMEM((D, S), BF16),
        pltpu.SemaphoreType.DMA((6 + S // TB + S // SB,)),
        pltpu.VMEM((D, S), F32),
        pltpu.VMEM((D + 2 * HP, D), BF16),
        pltpu.VMEM((D, DP), BF16),
        pltpu.VMEM((3 * D, D), BF16),
        pltpu.VMEM((D, DP), BF16),
        pltpu.VMEM((DP // 2, S), U32),
        pltpu.VMEM((S // 2, HP), U32),
        pltpu.VMEM((HP, S), BF16),
        pltpu.VMEM((S // 2, DP), U32),
        pltpu.VMEM((DP, S), BF16),
        pltpu.VMEM((DP, S), BF16),
        pltpu.VMEM((S, NQ), F32),
        pltpu.VMEM((NPB, S // 2, NQ), U32),
        pltpu.VMEM((4, 1, DP), F32),
        pltpu.VMEM((DH, (S // TB) * NVB, 128), F32),
        pltpu.VMEM((NPB, (DH + 1) * 8, 128), F32),
        pltpu.VMEM((1, 128), F32),
        pltpu.VMEM((1, NQ), F32),
        pltpu.VMEM((NPB, HP // 2, NQ), U32),
    ]
    out = pl.pallas_call(
        _kernel,
        out_shape=jax.ShapeDtypeStruct((D, S), BF16),
        in_specs=[pl.BlockSpec(memory_space=pl.ANY)] * 7,
        out_specs=pl.BlockSpec(memory_space=pl.ANY),
        scratch_shapes=scratch,
        compiler_params=pltpu.CompilerParams(vmem_limit_bytes=100 * 1024 * 1024),
    )(x, A_wq, A_wk.T, A_wv.T, A_wo, B_wqkv, B_wo)
    return out.T.reshape(1, S, D)
```
